```python
import os as _os
_os.environ.setdefault("JAX_PLATFORMS", "cpu")
import jax
import jax.numpy as jnp

def _softmax(x, axis=-1):
    return jax.nn.softmax(x, axis=axis)
def _gelu(x):
    return jax.nn.gelu(x, approximate=True)
def _silu(x):
    return jax.nn.silu(x)
def _sigmoid(x):
    return jax.nn.sigmoid(x)
def _layernorm(x, axis=-1, eps=1e-5):
    m = jnp.mean(x, axis=axis, keepdims=True)
    v = jnp.var(x, axis=axis, keepdims=True)
    return (x - m) / jnp.sqrt(v + eps)
def _scatter_add(tgt, idx, src, axis=0):
    return tgt.at[idx].add(src)
def _segment_sum(src, seg, n):
    return jax.ops.segment_sum(src, seg, n)
class _Rng:
    def __init__(self, key):
        self._k = key
    def _next(self):
        self._k, sub = jax.random.split(self._k)
        return sub
    def normal(self, shape):
        return jax.random.normal(self._next(), shape, dtype=jnp.bfloat16)
    def randint(self, lo, hi, shape):
        return jax.random.randint(self._next(), shape, lo, hi, dtype=jnp.int32)
    def uniform(self, shape, lo=0.0, hi=1.0):
        return jax.random.uniform(self._next(), shape, jnp.bfloat16, lo, hi)
    def permutation(self, n):
        return jax.random.permutation(self._next(), n)


kernel_name = 'standalone__grn__sampling'

def setup_inputs():
    _rng = _Rng(jax.random.key(int.from_bytes(__import__("os").urandom(4), "little")))
    _w = (lambda a: (lambda t: t.astype(jnp.bfloat16) if jnp.issubdtype(t.dtype, jnp.floating) else t)(jnp.asarray(a)))
    B, S, D = 512, 32, 640
    return {
        "x": _w((lambda *s: _rng.normal(s) * 0.05)(B, S, D)),
        "g": _w((lambda *s: _rng.normal(s) * 0.1)(D) * 0.1),
        "b": _w((lambda *s: _rng.normal(s) * 0.1)(D) * 0.1),
    }

def reference(x, g, b):
    gx = jnp.sqrt((x * x).sum(axis=-2, keepdims=True))
    nx = gx / (gx.mean(axis=-1, keepdims=True) + 1e-6)
    return g * (x * nx) + b + x
```

```python
import jax
import jax.numpy as jnp
import jax.experimental.pallas as pl
import jax.experimental.pallas.tpu as pltpu

_GROUPS = 8
_EPS = 1e-6


def _grn_kernel(x_hbm, g_hbm, b_hbm, o_hbm, buf, g_buf, b_buf, sems):
    groups, cols, _, _ = buf.shape
    head = (3 * cols) // 8
    last = cols - 1

    def read(k, lo, hi):
        window = pl.ds(lo, hi - lo)
        return pltpu.make_async_copy(x_hbm.at[:, window], buf.at[:, window], sems.at[k])

    def start_write(j):
        pltpu.make_async_copy(buf.at[:, j], o_hbm.at[:, j], sems.at[5]).start()

    read_head, read_body, read_tail = read(0, 0, head), read(1, head, last), read(2, last, cols)
    read_g = pltpu.make_async_copy(g_hbm, g_buf, sems.at[3])
    read_b = pltpu.make_async_copy(b_hbm, b_buf, sems.at[4])
    for copy in (read_head, read_g, read_b, read_body, read_tail):
        copy.start()

    read_g.wait()
    read_b.wait()
    g = g_buf[...].astype(jnp.float32).reshape(1, -1)
    b = b_buf[...].astype(jnp.float32).reshape(1, -1)

    def normalize(j):
        for q in range(groups):
            x = buf[q, j].astype(jnp.float32)
            gx = jnp.sqrt(jnp.sum(x * x, axis=0, keepdims=True))
            nx = gx / (jnp.mean(gx, axis=-1, keepdims=True) + _EPS)
            buf[q, j] = (x * (g * nx + 1.0) + b).astype(buf.dtype)

    read_head.wait()
    pl.loop(0, head)(normalize)

    read_body.wait()
    pl.loop(0, head)(start_write)

    read_tail.wait()

    @pl.loop(head, cols)
    def _(j):
        normalize(j)
        start_write(j)

    pltpu.make_async_copy(buf, buf, sems.at[5]).wait()


@jax.jit
def pallas_standalone__grn__sampling_kernel(x: jax.Array, g: jax.Array, b: jax.Array):
    B, S, D = x.shape
    view = (_GROUPS, B // _GROUPS, S, D)
    hbm = pl.BlockSpec(memory_space=pl.ANY)
    out = pl.pallas_call(
        _grn_kernel,
        in_specs=[hbm, hbm, hbm],
        out_specs=hbm,
        out_shape=jax.ShapeDtypeStruct(view, x.dtype),
        scratch_shapes=[
            pltpu.VMEM(view, x.dtype),
            pltpu.VMEM(g.shape, g.dtype),
            pltpu.VMEM(b.shape, b.dtype),
            pltpu.SemaphoreType.DMA((6,)),
        ],
        compiler_params=pltpu.CompilerParams(vmem_limit_bytes=64 * 1024 * 1024),
    )(x.reshape(view), g, b)
    return out.reshape(B, S, D)
```

```python
import jax
import jax.numpy as jnp
import jax.experimental.pallas as pl
import jax.experimental.pallas.tpu as pltpu

_STREAMS = 8
_EPS = 1e-6


def _grn_kernel(x_hbm, g_hbm, b_hbm, o_hbm, buf, g_buf, b_buf, sem_a, sem_b):
    streams, cols, rows, _ = buf.shape
    head = cols // 4
    last = cols - 1
    half = rows // 2

    def read_x(lo, hi, sem):
        window = pl.ds(lo, hi - lo)
        return pltpu.make_async_copy(x_hbm.at[:, window], buf.at[:, window], sem)

    def start_write(j):
        for r in (0, half):
            part = pl.ds(r, half)
            pltpu.make_async_copy(
                buf.at[:, j, part], o_hbm.at[:, j, part], sem_b
            ).start()

    first_reads = (
        read_x(0, head, sem_a),
        pltpu.make_async_copy(g_hbm, g_buf, sem_a),
        pltpu.make_async_copy(b_hbm, b_buf, sem_a),
    )
    read_body = read_x(head, last, sem_b)
    read_last = read_x(last, cols, sem_a)

    for copy in first_reads:
        copy.start()
    read_body.start()
    for copy in first_reads:
        copy.wait()
    read_last.start()

    g = g_buf[...].astype(jnp.float32).reshape(1, -1)
    b = b_buf[...].astype(jnp.float32).reshape(1, -1)

    def normalize(j):
        for s in range(streams):
            x = buf[s, j].astype(jnp.float32)
            gx = jnp.sqrt(jnp.sum(x * x, axis=0, keepdims=True))
            nx = gx / (jnp.mean(gx, axis=-1, keepdims=True) + _EPS)
            buf[s, j] = (x * (g * nx + 1.0) + b).astype(buf.dtype)

    pl.loop(0, head)(normalize)

    read_body.wait()
    pl.loop(0, head)(start_write)
    read_last.wait()

    @pl.loop(head, cols)
    def _(j):
        normalize(j)
        start_write(j)

    pltpu.make_async_copy(buf, o_hbm, sem_b).wait()


@jax.jit
def pallas_standalone__grn__sampling_kernel(
    x: jax.Array,
    g: jax.Array,
    b: jax.Array,
):
    batch, rows, channels = x.shape
    assert batch % _STREAMS == 0 and batch >= 4 * _STREAMS and rows % 32 == 0
    view = (_STREAMS, batch // _STREAMS, rows, channels)
    hbm = pl.BlockSpec(memory_space=pl.ANY)

    out = pl.pallas_call(
        _grn_kernel,
        in_specs=[hbm, hbm, hbm],
        out_specs=hbm,
        out_shape=jax.ShapeDtypeStruct(view, x.dtype),
        scratch_shapes=[
            pltpu.VMEM(view, x.dtype),
            pltpu.VMEM(g.shape, g.dtype),
            pltpu.VMEM(b.shape, b.dtype),
            pltpu.SemaphoreType.DMA,
            pltpu.SemaphoreType.DMA,
        ],
        compiler_params=pltpu.CompilerParams(
            vmem_limit_bytes=x.size * x.dtype.itemsize + 8 * 1024 * 1024
        ),
    )(x.reshape(view), g, b)
    return out.reshape(x.shape)
```
